```python
import os as _os
_os.environ.setdefault("JAX_PLATFORMS", "cpu")
import jax
import jax.numpy as jnp

def _softmax(x, axis=-1):
    return jax.nn.softmax(x, axis=axis)
def _gelu(x):
    return jax.nn.gelu(x, approximate=True)
def _silu(x):
    return jax.nn.silu(x)
def _sigmoid(x):
    return jax.nn.sigmoid(x)
def _layernorm(x, axis=-1, eps=1e-5):
    m = jnp.mean(x, axis=axis, keepdims=True)
    v = jnp.var(x, axis=axis, keepdims=True)
    return (x - m) / jnp.sqrt(v + eps)
def _scatter_add(tgt, idx, src, axis=0):
    return tgt.at[idx].add(src)
def _segment_sum(src, seg, n):
    return jax.ops.segment_sum(src, seg, n)
class _Rng:
    def __init__(self, key):
        self._k = key
    def _next(self):
        self._k, sub = jax.random.split(self._k)
        return sub
    def normal(self, shape):
        return jax.random.normal(self._next(), shape, dtype=jnp.bfloat16)
    def randint(self, lo, hi, shape):
        return jax.random.randint(self._next(), shape, lo, hi, dtype=jnp.int32)
    def uniform(self, shape, lo=0.0, hi=1.0):
        return jax.random.uniform(self._next(), shape, jnp.bfloat16, lo, hi)
    def permutation(self, n):
        return jax.random.permutation(self._next(), n)


kernel_name = 'sequential_preLN__mha_block__dense_activation_mish__prompt'

def setup_inputs():
    _rng = _Rng(jax.random.key(int.from_bytes(__import__("os").urandom(4), "little")))
    _w = (lambda a: (lambda t: t.astype(jnp.bfloat16) if jnp.issubdtype(t.dtype, jnp.floating) else t)(jnp.asarray(a)))
    def _A_setup():
        B, S, D, H = 1, 2048, 576, 32
        return {
            "x": _w((lambda *s: _rng.normal(s) * 0.05)(B, S, D)),
            "wqkv": _w((lambda *s: _rng.normal(s) * 0.05)(D, 3 * D)),
            "wo": _w((lambda *s: _rng.normal(s) * 0.05)(D, D)),
        }
    _A_in = _A_setup()

    def _B_setup():
        B, S, D, F = 1, 2048, 576, 4608
        return {
            "x": _w((lambda *s: _rng.normal(s) * 0.05)(B, S, D)),
            "w1": _w((lambda *s: _rng.normal(s) * 1.6)(D, F) * (D ** -0.5)),
            "b1": _w((lambda *s: _rng.normal(s) * 0.05)(F)),
            "w2": _w((lambda *s: _rng.normal(s) * 0.05)(F, D) * (F ** -0.5)),
        }
    _B_in = _B_setup()

    return {
        "A_x": _A_in["x"],
        "A_wqkv": _A_in["wqkv"],
        "A_wo": _A_in["wo"],
        "B_x": _B_in["x"],
        "B_w1": _B_in["w1"],
        "B_b1": _B_in["b1"],
        "B_w2": _B_in["w2"],
    }

def reference(A_x, A_wqkv, A_wo, B_x, B_w1, B_b1, B_w2):
    def _A_ref(x, wqkv, wo):
        B, S, D = x.shape
        H = 32
        Dh = D // H
        qkv = (lambda x, *d: x.transpose(*d))((x @ wqkv).reshape(B, S, 3, H, Dh), 2, 0, 3, 1, 4)
        q, k, v = qkv[0], qkv[1], qkv[2]
        scores = jnp.einsum("bhqd,bhkd->bhqk", q, k) * (Dh ** -0.5)
        p = _softmax(scores, axis=-1)
        o = jnp.einsum("bhqk,bhkd->bhqd", p, v)
        return (lambda x, *d: x.transpose(*d))(o, 0, 2, 1, 3).reshape(B, S, D) @ wo

    def _B_ref(x, w1, b1, w2):
        h = jnp.einsum("bsd,df->bsf", x, w1) + b1
        sp = jnp.log1p(jnp.exp(-jnp.abs(h))) + jnp.where(h > 0, h, jnp.zeros_like(h))
        act = h * jnp.tanh(sp)
        return jnp.einsum("bsf,fd->bsd", act, w2)

    x = A_x
    h = x + _A_ref(_layernorm(x, axis=-1), A_wqkv, A_wo)
    h2 = h + _B_ref(_layernorm(h, axis=-1), B_w1, B_b1, B_w2)
    return h2
```

```python
import functools
import math

import jax
import jax.numpy as jnp
from jax import lax
import jax.experimental.pallas as pl
import jax.experimental.pallas.tpu as pltpu

S = 2048
D = 576
H = 32
DH = 18
F = 4608
DP = 640
NW = 5
HW = 7
VR = 24
VP = 32
TQ = 512
NB = S // TQ
HG = 4
NG = H // HG
FC = 1536
LN_EPS = 1e-5
QSCALE = (DH ** -0.5) * math.log2(math.e)
M_MARGIN = 1.0 + 2.0 ** -6
L_THRESHOLD = 2.0 ** -64

f32 = jnp.float32
bf16 = jnp.bfloat16
i32 = jnp.int32


def _iota(shape, axis):
    return lax.broadcasted_iota(i32, shape, axis)


def _dot(a, b):
    return jnp.dot(a, b, preferred_element_type=f32)


def _dot_nt(a, b):
    return lax.dot_general(a, b, (((1,), (1,)), ((), ())), preferred_element_type=f32)


def _layernorm_t(xt):
    mu = jnp.mean(xt, axis=0, keepdims=True)
    xc = xt - mu
    var = jnp.mean(xc * xc, axis=0, keepdims=True)
    return xc * lax.rsqrt(var + LN_EPS)


def _mish(h):
    e = jnp.exp(jnp.minimum(h, 40.0))
    n = e * (e + 2.0)
    return h * (n / (n + 2.0))


def _kernel(x_hbm, wqkv_hbm, wo_hbm, w1_hbm, b1_hbm, w2t_hbm, out_hbm,
            x_v, wqkv_v, wo_v, w1_v, b1_v, w2t_v,
            wt_s, wpt, wot, qp, kp, vp, qn2, mbits, ot, outb,
            in_sem, x_sem, out_sem):
    def x_copy(c):
        return pltpu.make_async_copy(
            x_hbm.at[:, pl.ds(c * TQ, TQ)], x_v.at[:, pl.ds(c * TQ, TQ)], x_sem.at[c])

    cp_wqkv = pltpu.make_async_copy(wqkv_hbm, wqkv_v, in_sem.at[0])
    cp_wo = pltpu.make_async_copy(wo_hbm, wo_v, in_sem.at[1])
    cp_b1 = pltpu.make_async_copy(b1_hbm, b1_v, in_sem.at[2])
    cp_w1 = pltpu.make_async_copy(w1_hbm, w1_v, in_sem.at[3])
    cp_w2 = pltpu.make_async_copy(w2t_hbm, w2t_v, in_sem.at[4])

    cp_wqkv.start()
    for c in range(NB):
        x_copy(c).start()
    cp_wo.start()
    cp_b1.start()
    cp_w1.start()
    cp_w2.start()

    cp_wqkv.wait()
    wt_s[3 * D:, :] = jnp.zeros((wt_s.shape[0] - 3 * D, DP), f32)
    w_ext = jnp.concatenate(
        [wqkv_v[...].astype(f32), jnp.zeros((DP - D, 3 * D), f32)], axis=0)
    wt_s[0:3 * D, :] = w_ext.T

    row128 = _iota((128, DP), 0)
    col128 = _iota((128, DP), 1)
    for t in range(NW):
        nvalid = min(HW, H - HW * t) * DH
        qrows = wt_s[HW * DH * t:HW * DH * t + 128, :]
        wpt[128 * t:128 * (t + 1), :] = jnp.where(row128 < nvalid, qrows, 0.0).astype(bf16)
        krows = wt_s[D + HW * DH * t:D + HW * DH * t + 128, :]
        kone = jnp.where((row128 == 126) & (col128 == D), 1.0, 0.0)
        wpt[DP + 128 * t:DP + 128 * (t + 1), :] = jnp.where(row128 < nvalid, krows, kone).astype(bf16)
    row48 = _iota((2 * VR, DP), 0)
    col48 = _iota((2 * VR, DP), 1)
    vone = jnp.where(((row48 == DH) | (row48 == VR + DH)) & (col48 == D), 1.0, 0.0)
    vvalid = (row48 < DH) | ((row48 >= VR) & (row48 < VR + DH))
    for hp in range(H // 2):
        va = wt_s[2 * D + DH * (2 * hp):2 * D + DH * (2 * hp) + VR, :]
        vb = wt_s[2 * D + DH * (2 * hp + 1):2 * D + DH * (2 * hp + 1) + VR, :]
        vrows = jnp.concatenate([va, vb], axis=0)
        wpt[2 * DP + 2 * VR * hp:2 * DP + 2 * VR * (hp + 1), :] = (
            jnp.where(vvalid, vrows, vone).astype(bf16))

    gh = _iota((H, DP), 0)
    gr = _iota((H, DP), 1)
    g_t = (gh >= HW).astype(i32) + (gh >= 2 * HW).astype(i32) + \
          (gh >= 3 * HW).astype(i32) + (gh >= 4 * HW).astype(i32)
    g_lo = 128 * g_t + DH * (gh - HW * g_t)
    gmat = jnp.where((gr >= g_lo) & (gr < g_lo + DH), 1.0, 0.0).astype(bf16)

    ones_row = jnp.where(_iota((DP - D, TQ), 0) == 0, 1.0, 0.0).astype(bf16)
    kmax = jnp.zeros((H, TQ), f32)
    for c in range(NB):
        cs = slice(c * TQ, (c + 1) * TQ)
        x_copy(c).wait()
        xn = _layernorm_t(x_v[:, cs].astype(f32)).astype(bf16)
        xe = jnp.concatenate([xn, ones_row], axis=0)

        qb = (_dot(wpt[0:DP, :], xe) * QSCALE).astype(bf16)
        for t in range(NW):
            qp[t, :, cs] = qb[128 * t:128 * (t + 1), :]
        qf = qb.astype(f32)
        qn2[:, cs] = _dot(gmat, (qf * qf).astype(bf16))

        kf = _dot(wpt[DP:2 * DP, :], xe)
        kb = kf.astype(bf16)
        kr = kb.astype(f32)
        kmax = jnp.maximum(kmax, _dot(gmat, (kr * kr).astype(bf16)))
        for t in range(NW):
            kp[t, cs, :] = kr[128 * t:128 * (t + 1), :].T.astype(bf16)

        vf = _dot(wpt[2 * DP:, :], xe)
        vz = jnp.zeros((VP - VR, TQ), f32)
        for h in range(H):
            vp[h, :, cs] = jnp.concatenate([vf[VR * h:VR * (h + 1), :], vz], axis=0).astype(bf16)

    kmax2 = jnp.max(kmax, axis=1, keepdims=True)
    m_neg = -(jnp.sqrt(qn2[...] * kmax2) * M_MARGIN)
    m_neg = m_neg.astype(bf16).astype(f32)
    mbits[...] = lax.shift_right_logical(pltpu.bitcast(m_neg, i32), 16)

    cp_wo.wait()
    wot[...] = wo_v[...].astype(f32).T.astype(bf16)
    cp_b1.wait()
    cp_w1.wait()
    cp_w2.wait()

    word_row = _iota((64, TQ), 0)

    def head_rhs(h, qs, with_shift):
        t = h // HW
        lo = (DH // 2) * (h - HW * t)
        qw = pltpu.bitcast(qp[t, :, pl.ds(qs, TQ)], i32)
        if with_shift:
            mrow = mbits[pl.ds(h, 1), pl.ds(qs, TQ)]
            other = jnp.where(word_row == 63, mrow, 0)
        else:
            other = jnp.zeros((64, TQ), i32)
        rhs = jnp.where((word_row >= lo) & (word_row < lo + DH // 2), qw, other)
        return pltpu.bitcast(rhs, bf16), t

    def finish_head(g, i, o):
        l = o[DH:DH + 1, :]
        ot[g, DH * i:DH * (i + 1), :] = o[0:DH, :] / l
        return l

    def out_copy(b):
        bs = pl.ds(pl.multiple_of(b * TQ, TQ), TQ)
        return pltpu.make_async_copy(outb.at[:, bs], out_hbm.at[:, bs], out_sem.at[b])

    def block(b, carry):
        qs = pl.multiple_of(b * TQ, TQ)

        def group(g, lmin):
            ps = []
            for i in range(HG):
                rhs, t = head_rhs(g * HG + i, qs, True)
                ps.append(jnp.exp2(_dot(kp[t], rhs)).astype(bf16))
            for i in range(HG):
                o = _dot(vp[g * HG + i], ps[i])
                lmin = jnp.minimum(lmin, finish_head(g, i, o))
            return lmin

        lmin = lax.fori_loop(0, NG, group, jnp.full((1, TQ), jnp.inf, f32))

        @pl.when(jnp.logical_not(jnp.min(lmin) >= L_THRESHOLD))
        def _():
            def group_exact(g, c):
                for i in range(HG):
                    rhs, t = head_rhs(g * HG + i, qs, False)
                    s = _dot(kp[t], rhs)
                    m = jnp.max(s, axis=0, keepdims=True)
                    p = jnp.exp2(s - m).astype(bf16)
                    finish_head(g, i, _dot(vp[g * HG + i], p))
                return c
            lax.fori_loop(0, NG, group_exact, 0)

        ob = ot[...].reshape(D, TQ).astype(bf16)
        ht = x_v[:, pl.ds(qs, TQ)].astype(f32) + _dot(wot[...], ob)
        hn = _layernorm_t(ht).T.astype(bf16)

        acc = ht
        for j in range(F // FC):
            fs = slice(j * FC, (j + 1) * FC)
            hid = _dot(hn, w1_v[:, fs]) + b1_v[:, fs].astype(f32)
            acc = acc + _dot_nt(w2t_v[:, fs], _mish(hid).astype(bf16))
        outb[:, pl.ds(qs, TQ)] = acc.astype(outb.dtype)
        out_copy(b).start()
        return carry

    lax.fori_loop(0, NB, block, 0)
    for b in range(NB):
        out_copy(b).wait()


@jax.jit
def pallas_sequential_preLN__mha_block__dense_activation_mish__prompt_kernel(
    A_x: jax.Array,
    A_wqkv: jax.Array,
    A_wo: jax.Array,
    B_x: jax.Array,
    B_w1: jax.Array,
    B_b1: jax.Array,
    B_w2: jax.Array,
):
    del B_x
    xt = A_x.reshape(S, D).T
    w2t = B_w2.T
    b1 = B_b1.reshape(1, F)

    any_spec = pl.BlockSpec(memory_space=pl.ANY)
    out_t = pl.pallas_call(
        _kernel,
        out_shape=jax.ShapeDtypeStruct((D, S), A_x.dtype),
        in_specs=[any_spec] * 6,
        out_specs=any_spec,
        scratch_shapes=[
            pltpu.VMEM((D, S), bf16),
            pltpu.VMEM((D, 3 * D), bf16),
            pltpu.VMEM((D, D), bf16),
            pltpu.VMEM((D, F), bf16),
            pltpu.VMEM((1, F), bf16),
            pltpu.VMEM((D, F), bf16),
            pltpu.VMEM((3 * D + 64, DP), f32),
            pltpu.VMEM((2 * DP + H * VR, DP), bf16),
            pltpu.VMEM((D, D), bf16),
            pltpu.VMEM((NW, 128, S), bf16),
            pltpu.VMEM((NW, S, 128), bf16),
            pltpu.VMEM((H, VP, S), bf16),
            pltpu.VMEM((H, S), f32),
            pltpu.VMEM((H, S), i32),
            pltpu.VMEM((NG, HG * DH, TQ), f32),
            pltpu.VMEM((D, S), bf16),
            pltpu.SemaphoreType.DMA((5,)),
            pltpu.SemaphoreType.DMA((NB,)),
            pltpu.SemaphoreType.DMA((NB,)),
        ],
        compiler_params=pltpu.CompilerParams(vmem_limit_bytes=100 * 1024 * 1024),
        name="preln_mha_mish_block",
    )(xt, A_wqkv, A_wo, B_w1, b1, w2t)
    return out_t.T.reshape(1, S, D)
```

```python
import math

import jax
import jax.numpy as jnp
from jax import lax
import jax.experimental.pallas as pl
import jax.experimental.pallas.tpu as pltpu

S = 2048
D = 576
H = 32
DH = 18
F = 4608
NW = 5
HW = 7
VR = 24
WA = 384
WB = 1152
TQ = 512
NB = S // TQ
HG = 4
NG = H // HG
GPI = 2
NOUT = 4
KX = 128
KB = 128
FC = 512
LN_EPS = 1e-5
QSCALE = (DH ** -0.5) * math.log2(math.e)
M_MARGIN = 1.0 + 2.0 ** -6
L_THRESHOLD = 2.0 ** -80

f32 = jnp.float32
bf16 = jnp.bfloat16
i32 = jnp.int32


def _iota(shape, axis):
    return lax.broadcasted_iota(i32, shape, axis)


def _dot(a, b):
    return jnp.dot(a, b, preferred_element_type=f32)


def _dot_mixed(a, b):
    return lax.dot_general(a, b, (((1,), (0,)), ((), ())), preferred_element_type=f32)


def _dot_nt(a, b):
    return lax.dot_general(a, b, (((1,), (1,)), ((), ())), preferred_element_type=f32)


def _layernorm_t(xt):
    mu = jnp.mean(xt, axis=0, keepdims=True)
    xc = xt - mu
    var = jnp.mean(xc * xc, axis=0, keepdims=True)
    return xc * lax.rsqrt(var + LN_EPS)


def _mish(h):
    e = jnp.exp(jnp.minimum(h, 40.0))
    n = e * (e + 2.0)
    return h * (n / (n + 2.0))


def _kernel(x_hbm, wqkv_hbm, wo_hbm, w1_hbm, b1_hbm, w2t_hbm, out_hbm,
            x_v, wqkv_v, wo_v, w1_v, b1_v, w2t_v,
            b1r, wt_s, wot, qp, kp, vp, qn, mbits, p_a, p_b, ot, ot_exact, outb,
            in_sem, x_sem, out_sem):
    def x_copy(c):
        return pltpu.make_async_copy(
            x_hbm.at[:, pl.ds(c * TQ, TQ)], x_v.at[:, pl.ds(c * TQ, TQ)], x_sem.at[c])

    def w_copy(lo, hi, sem):
        return pltpu.make_async_copy(
            wqkv_hbm.at[:, pl.ds(lo, hi - lo)], wqkv_v.at[:, pl.ds(lo, hi - lo)], in_sem.at[sem])

    cp_wa = w_copy(0, WA, 0)
    cp_wb = w_copy(WA, WB, 5)
    cp_wc = w_copy(WB, 3 * D, 6)
    cp_wo = pltpu.make_async_copy(wo_hbm, wo_v, in_sem.at[1])
    cp_b1 = pltpu.make_async_copy(b1_hbm, b1_v, in_sem.at[2])
    cp_w1 = pltpu.make_async_copy(w1_hbm, w1_v, in_sem.at[3])
    cp_w2 = pltpu.make_async_copy(w2t_hbm, w2t_v, in_sem.at[4])

    x_copy(0).start()
    cp_wa.start()

    def ln1(c):
        return _layernorm_t(x_v[:, c * TQ:(c + 1) * TQ].astype(f32)).astype(bf16)

    gh = _iota((H, D // 2), 0)
    gw = _iota((H, D // 2), 1)
    gmat = jnp.where((gw >= (DH // 2) * gh) & (gw < (DH // 2) * (gh + 1)), 1.0, 0.0).astype(bf16)

    def head_sumsq(words):
        lo = pltpu.bitcast(lax.shift_left(words, 16), f32)
        hi = pltpu.bitcast(words & jnp.int32(-65536), f32)
        return _dot(gmat, (lo * lo + hi * hi).astype(bf16))

    qp[NW - 1] = jnp.zeros((64, S), i32)
    one_word = jnp.int32(0x3F80)
    wrow64 = _iota((64, TQ), 0)

    p_b[...] = jnp.ones((S, TQ), bf16)

    x_copy(0).wait()
    cp_wb.start()
    xn = ln1(0)
    cp_wa.wait()
    cp_wc.start()
    x_copy(1).start()
    cp_b1.start()
    wa_t = wqkv_v[:, 0:WA].T
    wt_s[0:WA, :] = wa_t

    def proj(lo, hi):
        return _dot(wt_s[lo:hi, :], xn)

    def cat(a, b):
        return jnp.concatenate([a, b], axis=0)

    kmax = jnp.zeros((H, TQ), f32)
    for c in range(NB):
        cs = slice(c * TQ, (c + 1) * TQ)

        if c == 0:
            q_lo = _dot(wa_t[0:D // 2], xn)
            cp_wb.wait()
            for cc in range(2, NB):
                x_copy(cc).start()
            cp_wo.start()
            wb_t = wqkv_v[:, WA:WB].T
            wt_s[WA:WB, :] = wb_t
            qf32 = cat(q_lo, _dot(cat(wa_t[D // 2:], wb_t[0:D - WA]), xn))
            k_lo = _dot(wb_t[D - WA:D - WA + D // 2], xn)
            cp_wc.wait()
            x_copy(1).wait()
            cp_b1.wait()
            wc_t = wqkv_v[:, WB:].T
            wt_s[WB:, :] = wc_t
            kf32 = cat(k_lo, proj(D + D // 2, 2 * D))
        else:
            qf32 = proj(0, D)
            kf32 = proj(D, 2 * D)

        if c == 1:
            for cc in range(2, NB):
                x_copy(cc).wait()
            cp_wo.wait()

        v_lo = proj(2 * D, 2 * D + D // 2)

        qb = (qf32 * QSCALE).astype(bf16)
        qw = pltpu.bitcast(qb, i32)
        for t in range(NW - 1):
            qp[t, :, cs] = qw[63 * t:63 * t + 64, :]
        qp[NW - 1, 0:D // 2 - 63 * (NW - 1), cs] = qw[63 * (NW - 1):, :]
        qn[:, cs] = jnp.sqrt(head_sumsq(qw)) * M_MARGIN

        kw = pltpu.bitcast(kf32.astype(bf16), i32)
        kmax = jnp.maximum(kmax, head_sumsq(kw))
        kw = cat(kw, jnp.zeros((64 * NW - D // 2, TQ), i32))
        for t in range(NW):
            win = jnp.where(wrow64 == 63, one_word, kw[63 * t:63 * t + 64, :])
            kp[t, cs, :] = pltpu.bitcast(win, bf16).T
        if c == NB - 1:
            kn = jnp.sqrt(jnp.max(kmax, axis=1, keepdims=True))
            m_neg = (-(qn[...] * kn)).astype(bf16).astype(f32)
            mbits[...] = lax.shift_right_logical(pltpu.bitcast(m_neg, i32), 16)
        if c == 1:
            wot[...] = wo_v[...].T
            cp_w1.start()
            cp_w2.start()
        if c == 2:
            b1f = b1_v[...].astype(f32)
            for r in range(F // 128):
                b1r[:, 128 * r:128 * (r + 1)] = b1f[r:r + 1, :]

        vf = cat(v_lo, proj(2 * D + D // 2, 3 * D)).astype(bf16).astype(f32)
        if c + 1 < NB:
            xn = ln1(c + 1)
        vf = cat(vf, jnp.zeros((8, TQ), f32))
        vrow = _iota((VR, TQ), 0)
        vfill = jnp.where(vrow == DH, 1.0, 0.0)
        for h in range(H):
            vp[h, :, cs] = jnp.where(vrow < DH, vf[DH * h:DH * h + VR, :], vfill)

    def head_rhs(h, qs, with_shift):
        t = sum((h >= HW * k).astype(i32) for k in range(1, NW))
        lo = (DH // 2) * (h - HW * t)
        qw = qp[t, :, pl.ds(qs, TQ)]
        if with_shift:
            mrow = mbits[pl.ds(h, 1), pl.ds(qs, TQ)]
            other = jnp.where(wrow64 == 63, mrow, 0)
        else:
            other = jnp.zeros((64, TQ), i32)
        rhs = jnp.where((wrow64 >= lo) & (wrow64 < lo + DH // 2), qw, other)
        return pltpu.bitcast(rhs, bf16), t

    def qk_pv_step(h_new, qs, p_new, h_old, p_old):
        rhs, t = head_rhs(h_new, qs, True)
        o = None
        for j in range(S // KB):
            js = slice(j * KB, (j + 1) * KB)
            oj = _dot_mixed(vp[h_old, :, js], p_old[js, :])
            o = oj if o is None else o + oj
            p_new[js, :] = jnp.exp2(_dot(kp[t, js, :], rhs)).astype(bf16)
        return o

    def finish_head(slot, i, o, unsafe):
        l = o[DH:DH + 1, :]
        ot[slot, DH * i:DH * (i + 1), :] = o[0:DH, :] / l
        return jnp.maximum(unsafe, jnp.where(l >= L_THRESHOLD, 0.0, 1.0))

    def attn_iter(it, unsafe):
        for gg in range(GPI):
            u = it * GPI + gg
            b = lax.shift_right_logical(u, 3)
            g = u & (NG - 1)
            qs = pl.multiple_of(b * TQ, TQ)
            for i in range(HG):
                p_new, p_old = (p_a, p_b) if i % 2 == 0 else (p_b, p_a)
                o = qk_pv_step(g * HG + i, qs, p_new, (g * HG + i - 1) & (H - 1), p_old)
                unsafe = finish_head(u if i == 0 else u + 1, (i - 1) % HG, o, unsafe)
        return unsafe

    unsafe = lax.fori_loop(0, NB * NG // GPI, attn_iter, jnp.zeros((1, TQ), f32))
    unsafe = finish_head(NB * NG, HG - 1, _dot_mixed(vp[H - 1], p_b[...]), unsafe)

    @pl.when(jnp.max(unsafe) > 0.0)
    def _():
        def exact_head(v, c):
            b = lax.shift_right_logical(v, 5)
            h = v & (H - 1)
            rhs, t = head_rhs(h, pl.multiple_of(b * TQ, TQ), False)

            def keys(j):
                return pl.ds(pl.multiple_of(j * KX, KX), KX)

            def max_step(j, m):
                s = _dot(kp[t, keys(j), :], rhs)
                return jnp.maximum(m, jnp.max(s, axis=0, keepdims=True))

            m = lax.fori_loop(0, S // KX, max_step, jnp.full((1, TQ), -jnp.inf, f32))

            def pv_step(j, o):
                s = _dot(kp[t, keys(j), :], rhs)
                return o + _dot_mixed(vp[h, :, keys(j)], jnp.exp2(s - m).astype(bf16))

            o = lax.fori_loop(0, S // KX, pv_step, jnp.zeros((VR, TQ), f32))
            ot_exact[h & (HG - 1)] = o / o[DH:DH + 1, :]

            @pl.when((h & (HG - 1)) == HG - 1)
            def _():
                slot = lax.shift_right_logical(v, 2) + 1
                for i in range(HG):
                    ot[slot, DH * i:DH * (i + 1), :] = ot_exact[i, 0:DH, :]
            return c
        lax.fori_loop(0, NB * H, exact_head, 0)

    cp_w1.wait()
    cp_w2.wait()

    RO = D // NOUT

    def out_copy(b, r):
        bs = pl.ds(pl.multiple_of(b * TQ, TQ), TQ)
        rs = slice(r * RO, (r + 1) * RO)
        return pltpu.make_async_copy(outb.at[rs, bs], out_hbm.at[rs, bs], out_sem.at[b, r])

    def block(b, carry):
        qs = pl.multiple_of(b * TQ, TQ)
        ob = ot[pl.ds(b * NG + 1, NG)].reshape(D, TQ).astype(bf16)
        ht = x_v[:, pl.ds(qs, TQ)].astype(f32) + _dot(wot[...], ob)
        hn = _layernorm_t(ht).T.astype(bf16)
        acc = ht
        for j in range(F // FC):
            fs = slice(j * FC, (j + 1) * FC)
            hid = _dot(hn, w1_v[:, fs]) + b1r[:, fs]
            act = _mish(hid).astype(bf16)
            if j + 1 < F // FC:
                acc = acc + _dot_nt(w2t_v[:, fs], act)
            else:
                for r in range(NOUT):
                    rs = slice(r * RO, (r + 1) * RO)
                    y = acc[rs, :] + _dot_nt(w2t_v[rs, fs], act)
                    outb[rs, pl.ds(qs, TQ)] = y.astype(outb.dtype)
                    out_copy(b, r).start()
        return carry

    lax.fori_loop(0, S // TQ, block, 0)
    for b in range(S // TQ):
        for r in range(NOUT):
            out_copy(b, r).wait()


@jax.jit
def pallas_sequential_preLN__mha_block__dense_activation_mish__prompt_kernel(
    A_x: jax.Array,
    A_wqkv: jax.Array,
    A_wo: jax.Array,
    B_x: jax.Array,
    B_w1: jax.Array,
    B_b1: jax.Array,
    B_w2: jax.Array,
):
    del B_x
    xt = A_x.reshape(S, D).T
    w2t = B_w2.T
    b1 = B_b1.reshape(F // 128, 128)

    any_spec = pl.BlockSpec(memory_space=pl.ANY)
    out_t = pl.pallas_call(
        _kernel,
        out_shape=jax.ShapeDtypeStruct((D, S), A_x.dtype),
        in_specs=[any_spec] * 6,
        out_specs=any_spec,
        scratch_shapes=[
            pltpu.VMEM((D, S), bf16),
            pltpu.VMEM((D, 3 * D), bf16),
            pltpu.VMEM((D, D), bf16),
            pltpu.VMEM((D, F), bf16),
            pltpu.VMEM((F // 128, 128), bf16),
            pltpu.VMEM((D, F), bf16),
            pltpu.VMEM((1, F), f32),
            pltpu.VMEM((3 * D, D), bf16),
            pltpu.VMEM((D, D), bf16),
            pltpu.VMEM((NW, 64, S), i32),
            pltpu.VMEM((NW, S, 128), bf16),
            pltpu.VMEM((H, VR, S), f32),
            pltpu.VMEM((H, S), f32),
            pltpu.VMEM((H, S), i32),
            pltpu.VMEM((S, TQ), bf16),
            pltpu.VMEM((S, TQ), bf16),
            pltpu.VMEM((NB * NG + 1, HG * DH, TQ), f32),
            pltpu.VMEM((HG, VR, TQ), f32),
            pltpu.VMEM((D, S), bf16),
            pltpu.SemaphoreType.DMA((7,)),
            pltpu.SemaphoreType.DMA((NB,)),
            pltpu.SemaphoreType.DMA((S // TQ, NOUT)),
        ],
        compiler_params=pltpu.CompilerParams(vmem_limit_bytes=100 * 1024 * 1024),
        name="preln_mha_mish_block",
    )(xt, A_wqkv, A_wo, B_w1, b1, w2t)
    return out_t.T.reshape(1, S, D)
```
